```python
import os as _os
_os.environ.setdefault("JAX_PLATFORMS", "cpu")
import jax
import jax.numpy as jnp

def _softmax(x, axis=-1):
    return jax.nn.softmax(x, axis=axis)
def _gelu(x):
    return jax.nn.gelu(x, approximate=True)
def _silu(x):
    return jax.nn.silu(x)
def _sigmoid(x):
    return jax.nn.sigmoid(x)
def _layernorm(x, axis=-1, eps=1e-5):
    m = jnp.mean(x, axis=axis, keepdims=True)
    v = jnp.var(x, axis=axis, keepdims=True)
    return (x - m) / jnp.sqrt(v + eps)
def _scatter_add(tgt, idx, src, axis=0):
    return tgt.at[idx].add(src)
def _segment_sum(src, seg, n):
    return jax.ops.segment_sum(src, seg, n)
class _Rng:
    def __init__(self, key):
        self._k = key
    def _next(self):
        self._k, sub = jax.random.split(self._k)
        return sub
    def normal(self, shape):
        return jax.random.normal(self._next(), shape, dtype=jnp.bfloat16)
    def randint(self, lo, hi, shape):
        return jax.random.randint(self._next(), shape, lo, hi, dtype=jnp.int32)
    def uniform(self, shape, lo=0.0, hi=1.0):
        return jax.random.uniform(self._next(), shape, jnp.bfloat16, lo, hi)
    def permutation(self, n):
        return jax.random.permutation(self._next(), n)


kernel_name = 'concat_heads__sliding_local_dilated__compressed_kv_cla__prompt'

def setup_inputs():
    _rng = _Rng(jax.random.key(int.from_bytes(__import__("os").urandom(4), "little")))
    _w = (lambda a: (lambda t: t.astype(jnp.bfloat16) if jnp.issubdtype(t.dtype, jnp.floating) else t)(jnp.asarray(a)))
    def _A_setup():
        B, S, D = 1, 2048, 640
        return {
            "x": _w((lambda *s: _rng.normal(s) * 0.2)(B, S, D)),
            "wqkv": _w((lambda *s: _rng.normal(s) * 0.2)(D, 3 * D)),
            "wo": _w((lambda *s: _rng.normal(s) * 0.05)(D, D)),
        }
    _A_in = _A_setup()

    def _B_setup():
        B, H, Sq, Sk, D, M = 1, 32, 2048, 2048, 128, 640
        Dc = 4 * D
        return {
            "x": _w((lambda *s: _rng.normal(s) * 0.8)(B, Sq, M)),
            "c_kv": _w((lambda *s: _rng.normal(s) * 0.8)(B, Sk, Dc)),
            "w_q": _w((lambda *s: _rng.normal(s) * 1.6)(M, H, D) * (M ** -0.5)),
            "w_uk": _w((lambda *s: _rng.normal(s) * 1.6)(Dc, H, D) * (Dc ** -0.5)),
            "w_uv": _w((lambda *s: _rng.normal(s) * 0.8)(Dc, H, D) * (Dc ** -0.5)),
            "w_o": _w((lambda *s: _rng.normal(s) * 0.8)(H, D, M) * ((H * D) ** -0.5)),
        }
    _B_in = _B_setup()

    return {
        "A_x": _A_in["x"],
        "A_wqkv": _A_in["wqkv"],
        "A_wo": _A_in["wo"],
        "B_x": _B_in["x"],
        "B_c_kv": _B_in["c_kv"],
        "B_w_q": _B_in["w_q"],
        "B_w_uk": _B_in["w_uk"],
        "B_w_uv": _B_in["w_uv"],
        "B_w_o": _B_in["w_o"],
    }

def reference(A_x, A_wqkv, A_wo, B_x, B_c_kv, B_w_q, B_w_uk, B_w_uv, B_w_o):
    def _A_ref(x, wqkv, wo):
        B, S, D = x.shape
        H = 32; Dh = D // H
        W, dil = 8, 2
        qkv = (lambda x, *d: x.transpose(*d))((x @ wqkv).reshape(B, S, 3, H, Dh), 2, 0, 3, 1, 4)
        q, k, v = qkv[0], qkv[1], qkv[2]
        scale = Dh ** -0.5
        pos = jnp.arange(S)
        off = jnp.arange(W) * dil
        idx = pos[:, None] - off[None, :]
        mask = idx >= 0
        idx_c = jnp.where(mask, idx, 0).reshape(-1)
        kg = k[:, :, idx_c, :].reshape(B, H, S, W, Dh)
        vg = v[:, :, idx_c, :].reshape(B, H, S, W, Dh)
        logits = jnp.einsum("bhsd,bhswd->bhsw", q, kg) * scale
        logits = jnp.where(mask[None, None, :, :], logits, -1e9)
        attn = _softmax(logits, axis=-1)
        o = jnp.einsum("bhsw,bhswd->bhsd", attn, vg)
        return (lambda x, *d: x.transpose(*d))(o, 0, 2, 1, 3).reshape(B, S, D) @ wo

    def _B_ref(x, c_kv, w_q, w_uk, w_uv, w_o):
        B, Sq, M = x.shape[0], x.shape[1], x.shape[2]
        Sk = c_kv.shape[1]
        H, D = w_q.shape[1], w_q.shape[2]
        q = jnp.einsum("bqm,mhd->bhqd", x, w_q)
        k = jnp.einsum("bkc,chd->bhkd", c_kv, w_uk)
        v = jnp.einsum("bkc,chd->bhkd", c_kv, w_uv)
        scores = jnp.einsum("bhqd,bhkd->bhqk", q, k) * (D ** -0.5)
        off = Sk - Sq
        qi = jnp.arange(Sq)[:, None]
        kj = jnp.arange(Sk)[None, :]
        cmask = kj <= (qi + off)
        scores = jnp.where(cmask[None, None], scores, -1e9)
        p = _softmax(scores, axis=-1)
        ctx = jnp.einsum("bhqk,bhkd->bhqd", p, v)
        return jnp.einsum("bhqd,hdm->bqm", ctx, w_o)

    a = _A_ref(A_x, A_wqkv, A_wo)
    b = _B_ref(B_x, B_c_kv, B_w_q, B_w_uk, B_w_uv, B_w_o)
    return jnp.concatenate([a, b], axis=-1)
```

```python
import functools

import jax
import jax.numpy as jnp
from jax import lax
import jax.experimental.pallas as pl
import jax.experimental.pallas.tpu as pltpu

S = 2048
DM = 640
DC = 512
HD = 128
NH = 32
BQ = 512
A_H, A_DH, A_W, A_DIL = 32, 20, 8, 2
CW = 512
PB = 512
SAFE_LOG2 = 64.0
SAFE_V = 2.0 ** 40
_ends = [4, 6, 8, 10, 12, 14, 15, 16, 22, 24, 26, 27, 28, 32]
CUTS = list(zip([0] + _ends[:-1], _ends))
A_PAD = 16
A_CH = 256
LOG2E = 1.4426950408889634
NT = (((1,), (1,)), ((), ()))
F32, BF16 = jnp.float32, jnp.bfloat16


def _dot(a, b):
    return jnp.dot(a, b, preferred_element_type=F32)


def _dot_nt(a, b):
    return lax.dot_general(a, b, NT, preferred_element_type=F32)


def _reorder_rows(x, n, wt_ref, wp_ref):
    wt_ref[n] = x
    for t in range(A_DH // 4):
        for d in range(4):
            wp_ref[n, pl.ds(128 * t + d, A_H, stride=4), :] = wt_ref[n, pl.ds(4 * t + d, A_H, stride=A_DH), :]
    return wp_ref[n].astype(BF16)


def _branch_a_in_weights(wqkv_ref, wt_ref, wp_ref, wqkv_t_ref, part):
    for n in range(DM // 128):
        blk = slice(128 * n, 128 * (n + 1))
        wqkv_t_ref[part, :, blk] = _reorder_rows(wqkv_ref[blk, part * DM:(part + 1) * DM].astype(F32).T, n, wt_ref, wp_ref)


def _branch_a_out_weights(wo_ref, wt_ref, wp_ref, wo_p_ref):
    for n in range(DM // 128):
        blk = slice(128 * n, 128 * (n + 1))
        wo_p_ref[:, blk] = _reorder_rows(wo_ref[:, blk].astype(F32), n, wt_ref, wp_ref)


def _branch_a_qkv(ax_ref, wqkv_t_ref, dst_refs, wait_x):
    for ref in dst_refs:
        ref[0:A_PAD, :] = jnp.zeros((A_PAD, DM), F32)

    def chunk(c, carry):
        wait_x(c)
        r0 = pl.multiple_of(c * A_CH, A_CH)
        for part, ref in enumerate(dst_refs):
            y = _dot_nt(ax_ref[pl.ds(r0, A_CH), :], wqkv_t_ref[part])
            ref[pl.ds(A_PAD + r0, A_CH), :] = y.astype(BF16).astype(F32)
        return carry

    lax.fori_loop(0, S // A_CH, chunk, 0)


def _windows(ref):
    win = {}
    for u in range(A_W // 2):
        x = ref[pl.ds(A_PAD - A_DIL * u - 8, A_CH + 8), :]
        win[u], win[u + A_W // 2] = x[8:], x[:A_CH]
    return [win[w] for w in range(A_W)]


def _branch_a_attend(q_ref, k_ref, v_ref, wo_ref, r0, fill):
    seg = (lax.broadcasted_iota(jnp.int32, (128, 128), 0) // 4
           == lax.broadcasted_iota(jnp.int32, (128, 128), 1) // 4)
    seg = jnp.where(seg, 1.0, 0.0).astype(BF16)
    q = q_ref[A_PAD:, :]
    row = lax.broadcasted_iota(jnp.int32, (A_CH, 128), 0) + r0
    lg = []
    for w, ks in enumerate(_windows(k_ref)):
        fill()
        part = functools.reduce(jnp.add, _lane_tiles(q * ks)).astype(BF16)
        lg.append(jnp.where(row >= A_DIL * w, _dot(part, seg) * (A_DH ** -0.5), -1e9))
    m = functools.reduce(jnp.maximum, lg)
    e = [jnp.exp(x - m) for x in lg]
    inv = 1.0 / functools.reduce(jnp.add, e)
    p = [x * inv for x in e]
    win = [_lane_tiles(x) for x in _windows(v_ref)]
    out = None
    for t in range(DM // 128):
        fill()
        o = functools.reduce(jnp.add, [x * vs[t] for x, vs in zip(p, win)])
        y = _dot(o.astype(BF16), wo_ref[128 * t:128 * (t + 1), :])
        out = y if out is None else out + y
    return out


def _lane_tiles(x):
    return [x[:, 128 * t:128 * (t + 1)] for t in range(x.shape[1] // 128)]


def _rows_from(x, r0, fn, y):
    if r0 == 0:
        return fn(x, y)
    return jnp.concatenate([x[:r0], fn(x[r0:], y)], axis=0)


def _weights(q_ref, k_ref, p_ref, l_ref, i):
    r0 = i * BQ
    l = None
    for c in range(r0 // CW):
        p = jnp.exp2(_dot_nt(q_ref[r0:r0 + BQ, :], k_ref[c * CW:(c + 1) * CW, :]))
        p_ref[:, c * CW:(c + 1) * CW] = p.astype(BF16)
        t = functools.reduce(jnp.add, _lane_tiles(p))
        l = t if l is None else l + t
    tri = (lax.broadcasted_iota(jnp.int32, (128, 128), 1)
           <= lax.broadcasted_iota(jnp.int32, (128, 128), 0))
    for j in range(BQ // 128):
        c0 = r0 + 128 * j
        p = jnp.exp2(_dot_nt(q_ref[c0:r0 + BQ, :], k_ref[c0:c0 + 128, :]))
        top = jnp.where(tri, p[:128], 0.0)
        p = top if p.shape[0] == 128 else jnp.concatenate([top, p[128:]], axis=0)
        p_ref[128 * j:, c0:c0 + 128] = p.astype(BF16)
        l = p if l is None else _rows_from(l, 128 * j, jnp.add, p)
    l_ref[...] = jnp.broadcast_to(jnp.sum(l, axis=1, keepdims=True), (BQ, 128))


def _attend_guarded(q_ref, k_ref, v_ref, ctx_ref):
    def block(b, carry):
        r0 = pl.multiple_of(b * 128, 128)
        s = _dot_nt(q_ref[pl.ds(r0, 128), :], k_ref[...])
        keep = (lax.broadcasted_iota(jnp.int32, (128, S), 1)
                <= lax.broadcasted_iota(jnp.int32, (128, S), 0) + r0)
        s = jnp.where(keep, s, -1e9 * LOG2E)
        p = jnp.exp2(s - jnp.max(s, axis=1, keepdims=True))
        o = _dot(p.astype(BF16), v_ref[...]) / jnp.sum(p, axis=1, keepdims=True)
        ctx_ref[pl.ds(r0, 128), :] = o.astype(BF16)
        return carry

    lax.fori_loop(0, S // 128, block, 0)


def _max_sq_norm(x):
    n = jnp.sum(x * x, axis=1, keepdims=True)
    return jnp.max(n, axis=0, keepdims=True)


def _values(v_ref, p_ref, l_ref, ctx_ref, i):
    r0 = i * BQ
    o = _dot(p_ref[:, 0:r0 + 128], v_ref[0:r0 + 128, :])
    for j in range(1, BQ // 128):
        c0 = r0 + 128 * j
        o = _rows_from(o, 128 * j, jnp.add, _dot(p_ref[128 * j:, c0:c0 + 128], v_ref[c0:c0 + 128, :]))
    ctx_ref[r0:r0 + BQ, :] = (o / l_ref[...]).astype(BF16)


def _head(w_ref, h):
    sh = (16 * (h % 2)).astype(jnp.uint32)
    return lax.bitcast_convert_type((w_ref[h // 2] >> sh) << 16, F32).astype(BF16)


def _kernel(ax_hbm, wqkv_hbm, wo_hbm, bx_hbm, c_hbm, wq_hbm, wk_hbm, wv_hbm, wbo_hbm, out_hbm,
            ax_ref, wqkv_ref, wo_ref, bx_ref, c_ref, wq_ref, wk_ref, wv_ref, wbo_ref, o_ref,
            qp_ref, kp_ref, vp_ref, wt_ref, wp_ref, wqkv_t_ref, wo_p_ref, q_ref, k_ref, v_ref, ctx_ref, p_ref, l_ref, sems, wsems, osems, isems, xsems):
    pairs = [(wo_hbm, wo_ref), (bx_hbm, bx_ref), (c_hbm, c_ref),
             (wbo_hbm, wbo_ref)]
    copies = [pltpu.make_async_copy(a, b, sems.at[n]) for n, (a, b) in enumerate(pairs)]

    def weight_copies(p):
        return [pltpu.make_async_copy(a.bitcast(jnp.uint32).at[:, p, :], b.at[p], wsems.at[n, p])
                for n, (a, b) in enumerate([(wq_hbm, wq_ref), (wk_hbm, wk_ref), (wv_hbm, wv_ref)])]

    def wqkv_copy(part):
        cols = pl.ds(part * DM, DM)
        return pltpu.make_async_copy(wqkv_hbm.at[:, cols], wqkv_ref.at[:, cols], isems.at[part])

    def x_copy(c):
        rows = pl.ds(pl.multiple_of(c * A_CH, A_CH), A_CH)
        return pltpu.make_async_copy(ax_hbm.at[rows, :], ax_ref.at[rows, :], xsems.at[c])

    for part in range(3):
        wqkv_copy(part).start()
    for part in range(3):
        wqkv_copy(part).wait()
        if part == 0:
            for c in range(S // A_CH):
                x_copy(c).start()
        _branch_a_in_weights(wqkv_ref, wt_ref, wp_ref, wqkv_t_ref, part)
    for cp in copies[:-1]:
        cp.start()
    for p in range(2):
        for cp in weight_copies(p):
            cp.start()
    _branch_a_qkv(ax_ref, wqkv_t_ref, (qp_ref, kp_ref, vp_ref), lambda c: x_copy(c).wait())
    for cp in copies[:-1]:
        cp.wait()
    copies[-1].start()

    nb = S // BQ

    def project(h):
        wq = _head(wq_ref, h)
        wkv = jnp.concatenate([_head(wk_ref, h), _head(wv_ref, h)], axis=1)
        qn, kn, vn = [], [], []
        for i in range(S // PB):
            rows = slice(i * PB, (i + 1) * PB)
            q = _dot(bx_ref[rows, :], wq) * (HD ** -0.5 * LOG2E)
            kv = _dot(c_ref[rows, :], wkv)
            q_ref[rows, :] = q.astype(BF16)
            k_ref[rows, :] = kv[:, :HD].astype(BF16)
            v_ref[rows, :] = kv[:, HD:].astype(BF16)
            qn.append(_max_sq_norm(q))
            kn.append(_max_sq_norm(kv[:, :HD]))
            vn.append(jnp.max(jnp.abs(kv[:, HD:]), axis=0, keepdims=True))
        qn, kn, vn = (functools.reduce(jnp.maximum, t) for t in (qn, kn, vn))
        ok = (qn * kn <= SAFE_LOG2 ** 2) & (jnp.max(vn, axis=1, keepdims=True) <= SAFE_V)
        return jnp.max(jnp.where(ok, 1.0, 0.0))

    def attend(h):
        _weights(q_ref, k_ref, p_ref.at[0], l_ref.at[0], 0)
        for i in range(nb):
            if i + 1 < nb:
                _weights(q_ref, k_ref, p_ref.at[(i + 1) % 2], l_ref.at[(i + 1) % 2], i + 1)
            _values(v_ref, p_ref.at[i % 2], l_ref.at[i % 2], ctx_ref.at[h], i)

    def attend_guarded(h):
        _attend_guarded(q_ref, k_ref, v_ref, ctx_ref.at[h])

    def head(h, safe):
        @pl.when(h % 2 == 1)
        def _():
            for cp in weight_copies((h + 1) // 2):
                cp.wait()

            @pl.when(h + 3 < NH)
            def _():
                for cp in weight_copies((h + 1) // 2 + 1):
                    cp.start()

        return lax.cond(safe > 0.5,
                        lambda: (attend(h), project(h + 1))[1],
                        lambda: (attend_guarded(h), project(h + 1))[1])

    for cp in weight_copies(0):
        cp.wait()
    _branch_a_out_weights(wo_ref, wt_ref, wp_ref, wo_p_ref)
    safe = lax.fori_loop(0, NH - 1, head, project(jnp.int32(0)))
    lax.cond(safe > 0.5, lambda: attend(NH - 1), lambda: attend_guarded(NH - 1))

    copies[-1].wait()

    def out_copy(n):
        rows = pl.ds(pl.multiple_of(n * A_CH, A_CH), A_CH)
        return pltpu.make_async_copy(o_ref.at[rows, :], out_hbm.at[rows, :], osems.at[n])

    def finish(n, carry):
        r0 = pl.multiple_of(n * A_CH, A_CH)
        rows = pl.ds(r0, A_CH)
        qv, kv, vv = (ref.at[pl.ds(r0, A_PAD + A_CH), :] for ref in (qp_ref, kp_ref, vp_ref))

        def proj_o(h0, h1):
            ctx = jnp.concatenate([ctx_ref[h, rows, :] for h in range(h0, h1)], axis=1)
            return _dot(ctx, wbo_ref[h0 * HD:h1 * HD, :])

        cuts = iter(CUTS)
        ob = []

        def fill():
            h0, h1 = next(cuts)
            ob.append(proj_o(h0, h1))

        o_ref[rows, :DM] = _branch_a_attend(qv, kv, vv, wo_p_ref, r0, fill).astype(BF16)
        fill()
        o_ref[rows, DM:] = functools.reduce(jnp.add, ob).astype(BF16)
        out_copy(n).start()
        return carry

    lax.fori_loop(0, S // A_CH, finish, 0)
    for n in range(S // A_CH):
        out_copy(n).wait()


@jax.jit
def pallas_concat_heads__sliding_local_dilated__compressed_kv_cla__prompt_kernel(
    A_x, A_wqkv, A_wo, B_x, B_c_kv, B_w_q, B_w_uk, B_w_uv, B_w_o,
):
    hbm = pl.BlockSpec(memory_space=pltpu.HBM)
    vm = pltpu.VMEM
    out = pl.pallas_call(
        _kernel,
        in_specs=[hbm] * 9,
        out_specs=hbm,
        out_shape=jax.ShapeDtypeStruct((S, 2 * DM), BF16),
        scratch_shapes=[
            vm((S, DM), BF16), vm((DM, 3 * DM), BF16), vm((DM, DM), BF16),
            vm((S, DM), BF16), vm((S, DC), BF16),
            vm((NH // 2, DM, HD), jnp.uint32), vm((NH // 2, DC, HD), jnp.uint32), vm((NH // 2, DC, HD), jnp.uint32), vm((NH * HD, DM), BF16),
            vm((S, 2 * DM), BF16),
            vm((S + A_PAD, DM), F32), vm((S + A_PAD, DM), F32), vm((S + A_PAD, DM), F32),
            vm((DM // 128, DM, 128), F32), vm((DM // 128, DM, 128), F32), vm((3, DM, DM), BF16), vm((DM, DM), BF16),
            vm((S, HD), BF16), vm((S, HD), BF16), vm((S, HD), BF16), vm((NH, S, HD), BF16),
            vm((2, BQ, S), BF16), vm((2, BQ, 128), F32),
            pltpu.SemaphoreType.DMA((4,)), pltpu.SemaphoreType.DMA((3, NH // 2)),
            pltpu.SemaphoreType.DMA((S // A_CH,)), pltpu.SemaphoreType.DMA((3,)),
            pltpu.SemaphoreType.DMA((S // A_CH,)),
        ],
        compiler_params=pltpu.CompilerParams(vmem_limit_bytes=120 * 1024 * 1024, flags={"XLA_TPU_EVENLY_DISTRIBUTE_CRITICAL_NODES": True}),
    )(A_x.reshape(S, DM), A_wqkv, A_wo, B_x.reshape(S, DM), B_c_kv.reshape(S, DC),
      B_w_q, B_w_uk, B_w_uv, B_w_o.reshape(NH * HD, DM))
    return out.reshape(1, S, 2 * DM)
```
